```python
import jax
import jax.numpy as jnp

def _softmax(x, axis=-1):
    return jax.nn.softmax(x, axis=axis)
def _gelu(x):
    return jax.nn.gelu(x, approximate=True)
def _silu(x):
    return jax.nn.silu(x)
def _sigmoid(x):
    return jax.nn.sigmoid(x)
def _layernorm(x, axis=-1, eps=1e-5):
    m = jnp.mean(x, axis=axis, keepdims=True)
    v = jnp.var(x, axis=axis, keepdims=True)
    return (x - m) / jnp.sqrt(v + eps)
def _scatter_add(tgt, idx, src, axis=0):
    return tgt.at[idx].add(src)
def _segment_sum(src, seg, n):
    return jax.ops.segment_sum(src, seg, n)
class _Rng:
    def __init__(self, key):
        self._k = key
    def _next(self):
        self._k, sub = jax.random.split(self._k)
        return sub
    def normal(self, shape):
        return jax.random.normal(self._next(), shape, dtype=jnp.bfloat16)
    def randint(self, lo, hi, shape):
        return jax.random.randint(self._next(), shape, lo, hi, dtype=jnp.int32)
    def uniform(self, shape, lo=0.0, hi=1.0):
        return jax.random.uniform(self._next(), shape, jnp.bfloat16, lo, hi)
    def permutation(self, n):
        return jax.random.permutation(self._next(), n)


kernel_name = 'parallel_sum__linear_kernel_hedgehog__glu_gated_geglu__prompt'

def _fwd_setup_inputs():
    _rng = _Rng(jax.random.key(int.from_bytes(__import__("os").urandom(4), "little")))
    _w = (lambda a: (lambda t: t.astype(jnp.bfloat16) if jnp.issubdtype(t.dtype, jnp.floating) else t)(jnp.asarray(a)))
    def _A_setup():
        B, S, D, H = 1, 2048, 448, 16
        Dh = D // H
        return {
            "x": _w((lambda *s: _rng.normal(s) * 0.05)(B, S, D)),
            "wqkv": _w((lambda *s: _rng.normal(s) * 0.05)(D, 3 * D)),
            "w_phi": _w((lambda *s: _rng.normal(s) * 0.05)(H, Dh, Dh) * (Dh ** -0.5)),
            "wo": _w((lambda *s: _rng.normal(s) * 0.05)(D, D)),
        }
    _A_in = _A_setup()

    def _B_setup():
        B, S, Dm, Df = 1, 2048, 448, 1792
        return {
            "x": _w((lambda *s: _rng.normal(s) * 0.05)(B, S, Dm)),
            "w_gate": _w((lambda *s: _rng.normal(s) * 0.05)(Dm, Df) * (Dm ** -0.5)),
            "w_up": _w((lambda *s: _rng.normal(s) * 0.05)(Dm, Df) * (Dm ** -0.5)),
            "w_down": _w((lambda *s: _rng.normal(s) * 0.05)(Df, Dm) * (Df ** -0.5)),
        }
    _B_in = _B_setup()

    return {
        "A_x": _A_in["x"],
        "A_wqkv": _A_in["wqkv"],
        "A_w_phi": _A_in["w_phi"],
        "A_wo": _A_in["wo"],
        "B_x": _B_in["x"],
        "B_w_gate": _B_in["w_gate"],
        "B_w_up": _B_in["w_up"],
        "B_w_down": _B_in["w_down"],
    }

def _fwd_reference(A_x, A_wqkv, A_w_phi, A_wo, B_x, B_w_gate, B_w_up, B_w_down):
    def _A_ref(x, wqkv, w_phi, wo):
        B, S, D = x.shape
        H = 16; Dh = D // H
        qkv = (lambda x, *d: x.transpose(*d))((x @ wqkv).reshape(B, S, 3, H, Dh), 2, 0, 3, 1, 4)
        q, k, v = qkv[0], qkv[1], qkv[2]
        pq = jnp.einsum("bhsd,hdf->bhsf", q, w_phi)
        pk = jnp.einsum("bhsd,hdf->bhsf", k, w_phi)
        phi_q = jnp.concatenate([_softmax(pq, axis=-1), _softmax(-pq, axis=-1)], axis=-1)
        phi_k = jnp.concatenate([_softmax(pk, axis=-1), _softmax(-pk, axis=-1)], axis=-1)
        kv = jnp.einsum("bhsf,bhsd->bhfd", phi_k, v)
        z  = jnp.einsum("bhsf->bhf", phi_k)
        num = jnp.einsum("bhqf,bhfd->bhqd", phi_q, kv)
        den = jnp.einsum("bhqf,bhf->bhq", phi_q, z)[..., None] + 1e-6
        o = num / den
        return (lambda x, *d: x.transpose(*d))(o, 0, 2, 1, 3).reshape(B, S, D) @ wo

    def _B_ref(x, w_gate, w_up, w_down):
        g = jnp.einsum("bsd,df->bsf", x, w_gate)
        u = jnp.einsum("bsd,df->bsf", x, w_up)
        h = _gelu(g) * u
        return jnp.einsum("bsf,fd->bsd", h, w_down)

    x = A_x
    xn = _layernorm(x, axis=-1)
    return x + _A_ref(xn, A_wqkv, A_w_phi, A_wo) + _B_ref(xn, B_w_gate, B_w_up, B_w_down)


def setup_inputs():
    _inp = _fwd_setup_inputs()
    _gk = jax.random.fold_in(jax.random.key(int.from_bytes(__import__("os").urandom(4), "little")), 2**31 - 1)
    _shapes = [[1, 2048, 448]]
    _dtypes = ['bfloat16']
    _gks = jax.random.split(_gk, len(_shapes))
    _gs = [jax.random.normal(k, s, dtype=jnp.dtype(d)) * 0.05 for k, s, d in zip(_gks, _shapes, _dtypes)]
    _inp["grad_out"] = _gs[0]
    return _inp

def reference(A_x, A_wqkv, A_w_phi, A_wo, B_w_gate, B_w_up, B_w_down, B_x, grad_out):
    _const = dict(B_x=B_x)
    def _f(*_d):
        return _fwd_reference(**{'A_x': _d[0], 'A_wqkv': _d[1], 'A_w_phi': _d[2], 'A_wo': _d[3], 'B_w_gate': _d[4], 'B_w_up': _d[5], 'B_w_down': _d[6], **_const})
    _out, _vjp = jax.vjp(_f, A_x, A_wqkv, A_w_phi, A_wo, B_w_gate, B_w_up, B_w_down)
    _grads = _vjp(grad_out)
    _out0 = jnp.asarray(_out)
    return (_out0, *[jnp.asarray(_g) for _g in _grads])
```

```python
import functools

import jax
import jax.numpy as jnp
import jax.experimental.pallas as pl
import jax.experimental.pallas.tpu as pltpu

S, D, F, H, DH = 2048, 448, 1792, 16, 28
TC = 512
NC = S // TC
FC = 256
NF = F // FC
NP = 8
PR = 56
bf16 = jnp.bfloat16
f32 = jnp.float32
u32 = jnp.uint32

NN = (((1,), (0,)), ((), ()))
NT = (((1,), (1,)), ((), ()))

C0 = 0.7978845608028654
C1 = 0.044715
LOG2E = 1.4426950408889634


def dot(a, b, dn=NN):
    return jax.lax.dot_general(a, b, dn, preferred_element_type=f32)


def iota(shape, dim):
    return jax.lax.broadcasted_iota(jnp.int32, shape, dim)


def geglu_fwd_bwd(g, u, dh):
    g2 = g * g
    t = jnp.tanh(g * (C0 + (C0 * C1) * g2))
    cdf = 0.5 * t + 0.5
    gl = g * cdf
    dgl = cdf + (0.5 * g) * (1.0 - t * t) * (C0 + (3.0 * C0 * C1) * g2)
    return gl * u, dh * u * dgl, dh * gl


def pair_reduce(x, op):
    a = x[0:8]
    for i in range(1, 7):
        a = op(a, x[8 * i:8 * i + 8])
    a = op(a, pltpu.roll(a, 2, 0))
    return op(a, pltpu.roll(a, 4, 0))


def recip(s):
    r = pl.reciprocal(s, approx=True)
    return r * (2.0 - s * r)


def rep7(a):
    return jnp.concatenate([a] * 7, axis=0)


def hedgehog(p):
    ep = jnp.exp2(p - rep7(pair_reduce(p, jnp.maximum)))
    en = jnp.exp2(rep7(pair_reduce(p, jnp.minimum)) - p)
    ep = ep * rep7(recip(pair_reduce(ep, jnp.add)))
    en = en * rep7(recip(pair_reduce(en, jnp.add)))
    return jnp.concatenate([ep, en], axis=0)


def hedgehog_bwd(phi, dphi):
    t = phi * dphi
    tp, tn = t[0:PR], t[PR:2 * PR]
    sp = rep7(pair_reduce(tp, jnp.add))
    sn = rep7(pair_reduce(tn, jnp.add))
    return (tp - tn) - (phi[0:PR] * sp - phi[PR:2 * PR] * sn)


def kv_masks():
    row = iota((64, 112), 0)
    par = iota((64, 112), 1) & 1
    row_head = jnp.where(row < PR, (row >= DH).astype(jnp.int32), (row >= 60).astype(jnp.int32))
    full = row_head == par
    single = jnp.logical_and(full, jnp.logical_or(row < PR, (row & 3) == 3))
    return full, single


def quad_maps():
    def head_of_c(c):
        return (c >= 28).astype(jnp.int32) + (c >= 56).astype(jnp.int32) + (c >= 84).astype(jnp.int32)

    def head_of_r(r):
        return 2 * (r >= PR).astype(jnp.int32) + (r & 1)

    def f_of_r(r):
        return (r - PR * (r >= PR).astype(jnp.int32)) >> 1

    mask_cr = head_of_c(iota((112, 112), 0)) == head_of_r(iota((112, 112), 1))
    mask_rc = head_of_r(iota((112, 112), 0)) == head_of_c(iota((112, 112), 1))
    e_rf = jnp.where(f_of_r(iota((112, DH), 0)) == iota((112, DH), 1), 1.0, 0.0).astype(bf16)
    return mask_cr, mask_rc, e_rf


ALPHA = (((0, 1), (3, 1)), ((2, 1), (3, 1)), ((0, 1),), ((3, 1),), ((0, 1), (1, 1)), ((2, 1), (0, -1)), ((1, 1), (3, -1)))
BETA = (((0, 1), (3, 1)), ((0, 1),), ((1, 1), (3, -1)), ((2, 1), (0, -1)), ((3, 1),), ((0, 1), (1, 1)), ((2, 1), (3, 1)))
GAMMA = (((0, 1), (3, 1)), ((2, 1), (3, -1)), ((1, 1), (3, 1)), ((0, 1), (2, 1)), ((1, 1), (0, -1)), ((3, 1),), ((0, 1),))
R7 = tuple(range(7))


def signed_sum(terms):
    acc, sg = terms[0]
    for v, s in terms[1:]:
        if s == sg:
            acc = acc + v
        elif sg > 0:
            acc = acc - v
        else:
            acc, sg = v - acc, 1
    assert sg > 0
    return acc


def spread(tab, g, n):
    if n == 1:
        return [g[0, 0]]
    h = n // 2
    out = []
    for row in tab:
        sub = {(i, j): signed_sum([(g[h * (q >> 1) + i, h * (q & 1) + j], s) for q, s in row])
               for i in range(h) for j in range(h)}
        out += spread(tab, sub, h)
    return out


def gather(tab, m, n, orders=(R7, R7)):
    if n == 1:
        return {(0, 0): m[0]}
    h = n // 2
    k = len(m) // 7
    subs = [gather(tab, m[k * r:k * (r + 1)], h, orders[1:]) for r in range(7)]
    out = {}
    for q in range(4):
        for i in range(h):
            for j in range(h):
                out[h * (q >> 1) + i, h * (q & 1) + j] = signed_sum(
                    [(subs[r][i, j], s) for r in orders[0] for qq, s in tab[r] if qq == q])
    return out


def grid(x, n, swap):
    r, c = x.shape[0] // n, x.shape[1] // n
    return {((j, i) if swap else (i, j)): x[r * i:r * (i + 1), c * j:c * (j + 1)]
            for i in range(n) for j in range(n)}


def ungrid(g, n, swap):
    return jnp.concatenate(
        [jnp.concatenate([g[(j, i) if swap else (i, j)] for j in range(n)], axis=1) for i in range(n)], axis=0)


def pk(x):
    return pltpu.bitcast(x.astype(bf16), u32)


def up(x):
    return pltpu.bitcast(x, bf16)


def total(xs):
    acc = xs[0]
    for x in xs[1:]:
        acc = acc + x
    return acc


OPT_ASEQ = (1, 1, 1, 1, 1, 1, 1, 1, 1, 1, 1, 1, 1, 1, 1, 1, 0, 0, 0, 0, 0, 0, 0, 0, 0, 0, 0, 0, 0, 0, 0, 0, 2, 2, 2, 2, 2, 2, 2, 2, 2, 2, 2, 2, 2, 2, 2, 2, 4, 4, 4, 4, 4, 4, 4, 4)
OPT_BM = (112, 112)
OPT_BO = (1, 5, 0, 2, 4, 6, 3)
OPT_BP = (0, 4, 1, 5, 2, 6, 3, 7)
OPT_BQ = (0, 4, 1, 5, 2, 6, 3, 7)
OPT_BR = 10
OPT_BS = 'nnnndndndndndkdkdkdkakakakakaaaa'
OPT_BT = 4
OPT_C0 = 0
OPT_C1 = 7
OPT_C2 = 50
OPT_C3 = 1250
OPT_CI = (1, 5, 0, 2, 4, 6, 3)
OPT_CM = (48, 32, 32)
OPT_CO = (1, 5, 4, 6, 0, 2, 3)
OPT_DM = 448
OPT_EO = (0, 5, 6, 3, 1, 2, 4)
OPT_ES = 'ffbfbfbfbfbfbfbfbfbbfbbfbbfbbfbbfbbfbbfbbfbbfbbfbbfbbffofpffff'
OPT_F0 = 800
OPT_F1 = 4000
OPT_F4 = 1000
OPT_F5 = 3700
OPT_FI = (4, 2, 0, 3, 1, 6, 5)
OPT_FO = 'd0 g0 d4 g4 d3 g3 d6 g6 d2 g2 d1 d5 g1 g5'
OPT_FS = 'f00123 f10123 f20123 x00123 f30123 x10123 w001234567 x20123 x30123 p w101234567'
OPT_G0 = 0
OPT_G1 = 5200
OPT_G4 = 3700
OPT_G5 = 4700
OPT_G6 = 0
OPT_G7 = 150
OPT_G8 = 3600
OPT_G9 = 5300
OPT_GL = 6
OPT_P0 = 300
OPT_P1 = 800
OPT_P2 = 1600
OPT_P3 = 0
OPT_P4 = 800
OPT_PX = 2
OPT_Q0 = 0
OPT_Q1 = 0
OPT_Q2 = 500
OPT_Q3 = 3300
OPT_Q4 = 0
OPT_Q5 = 0
OPT_Q6 = 300
OPT_Q7 = 3000

SEM_EVEN, SEM_ODD, SEM_GROUP, SEM_OUT, SEM_X = range(5)
NSEM = 5

Q4 = 112
D2 = 224
MS = 32
XCUT = (0, 5, 18, 37, 56)
WCUT = (0, 10, 20, 30, 39, 49, 51, 54, 56)
PAIRS = (0, 2, 4, 6, 1, 3, 5, 7)


def kernel(x_h, dy_h, wqkv_h, wphi_h, wo_h, wg_h, wu_h, wd_h,
           out_h, dx_h, dwqkv_h, dwphi_h, dwo_h, dwg_h, dwu_h, dwd_h,
           x_s, dy_s, wqkv_s, wphi_s, wo_s, wgu_s, wd_s,
           out_s, dx_s, dwq_s, dwphi_s, dwo_s, dwgu_s, dwd_s,
           ax_s, ay_s, co_s, stat_s, do_s, phq_s, phk_s, vext_s,
           accx, acco, g_acc, kv_acc, dkv_acc, kvm_s, kvT_s, dkvm_s, dkvT_s,
           bg_s, bgT_s, bd_s, bdT_s, bq_s, bo_s,
           wT_s, blk_s, xa_s, xb_s, xn_s, wop_s, wpT_s, wp_s, woT_s, wf_s, dwo_acc,
           sem):

    always = [None]

    def cp(src, dst, k):
        return pltpu.make_async_copy(src, dst, sem.at[k])

    def tok(i):
        return pl.ds(pl.multiple_of(i * TC, TC), TC)

    def fcol(j):
        return pl.ds(pl.multiple_of(j * FC, FC), FC)

    def wsem(j):
        if isinstance(j, int):
            return SEM_GROUP if j == 0 else j & 1
        return jnp.where(j == 0, SEM_GROUP, j & 1)

    cp_x = lambda i, k=SEM_X: cp(x_h.at[:, tok(i)], x_s.at[i], k)
    cp_dy = lambda i, k=SEM_GROUP: cp(dy_h.at[:, tok(i)], dy_s.at[i], k)
    cp_wqkv = lambda d: cp(wqkv_h.at[pl.ds(Q4 * d, Q4)], wqkv_s[d], SEM_OUT)
    cp_wphi = lambda: cp(wphi_h, wphi_s, SEM_GROUP)
    cp_wo = lambda: cp(wo_h, wo_s, SEM_EVEN)
    cp_wg = lambda j: cp(wg_h.at[:, fcol(j)], wgu_s.at[j, :, pl.ds(0, FC)], wsem(j))
    cp_wu = lambda j: cp(wu_h.at[:, fcol(j)], wgu_s.at[j, :, pl.ds(FC, FC)], wsem(j))
    cp_wd = lambda j: cp(wd_h.at[:, fcol(j)], wd_s.at[j], wsem(j))
    cp_out = lambda i: cp(out_s.at[i], out_h.at[:, tok(i)], SEM_OUT)
    cp_dx = lambda i: cp(dx_s.at[i], dx_h.at[:, tok(i)], SEM_OUT)
    cp_dwg = lambda j: cp(dwgu_s.at[j, :, pl.ds(0, FC)], dwg_h.at[:, fcol(j)], SEM_OUT)
    cp_dwu = lambda j: cp(dwgu_s.at[j, :, pl.ds(FC, FC)], dwu_h.at[:, fcol(j)], SEM_OUT)
    cp_dwd = lambda j: cp(dwd_s.at[j], dwd_h.at[:, fcol(j)], SEM_OUT)
    cp_dwqkv = lambda d: cp(dwq_s[d], dwqkv_h.at[pl.ds(Q4 * d, Q4)], SEM_OUT)
    cp_dwphi = lambda: cp(dwphi_s, dwphi_h, SEM_OUT)
    cp_dwo = lambda m: cp(dwo_s[m], dwo_h.at[pl.ds(Q4 * m, Q4)], SEM_OUT)

    def gated(v, tok):
        if tok is None:
            return v
        if tok.dtype != v.dtype:
            tok = pltpu.bitcast(tok, v.dtype)
        rows = []
        for r in range(0, v.shape[0], 8):
            cols = []
            for c in range(0, v.shape[1], 128):
                w = min(128, v.shape[1] - c)
                k = min(w, tok.shape[1])
                cols.append(jnp.where(always[0][:, 0:k] >= 0, v[r:r + 8, c:c + k], tok[:, 0:k]))
                if k < w:
                    cols.append(v[r:r + 8, c + k:c + w])
            rows.append(jnp.concatenate(cols, axis=1))
        return jnp.concatenate(rows, axis=0)

    def ln_stats(i, t, tok=None):
        lanes = pl.ds(128 * t, 128)
        slab = lambda k: x_s[i, pl.ds(16 * k, 16), lanes].astype(f32)
        fold = lambda a: jnp.sum(a[0:8] + a[8:16], axis=0, keepdims=True) * (1.0 / D)
        x0 = slab(0)
        shift = jnp.broadcast_to(x0[0:1], (16, 128))
        s1 = x0 - shift
        s2 = s1 * s1
        for k in range(1, D // 16):
            xk = slab(k) - shift
            s1 = s1 + xk
            s2 = s2 + xk * xk
        m = fold(s1)
        var = jnp.maximum(fold(s2) - m * m, 0.0)
        stat_s[i, 0, :, lanes] = gated(jnp.broadcast_to(x0[0:1] + m, (8, 128)), tok)
        stat_s[i, 1, :, lanes] = gated(jnp.broadcast_to(jax.lax.rsqrt(var + 1e-5), (8, 128)), tok)

    def xn_rows(i, r0, mu, rstd):
        return (x_s[i, pl.ds(r0, 16), :].astype(f32) - mu) * rstd

    def ld_stats(i):
        return [jnp.concatenate([stat_s[i, k]] * 2, axis=0) for k in range(2)]

    def ax_jobs(i):
        c = {}

        def slab(sl):
            if not c:
                c["stats"] = ld_stats(i)
            g = {}
            for d in range(4):
                xn = xn_rows(i, Q4 * d + 16 * sl, *c["stats"])
                for t in range(4):
                    g[t, d] = xn[:, 128 * t:128 * (t + 1)]
            c[sl] = [store_job(ax_s, (i, r, pl.ds(8 * sl, 8), slice(None)), pk(a))
                     for r, a in enumerate(spread(ALPHA, g, 4))]

        def run(sl, n, tok):
            if n == 0:
                slab(sl)
            c[sl][n](tok)
        return [functools.partial(run, sl, n) for sl in range(7) for n in range(49)]

    def ln_slab(i, k, tok):
        xn_s[pl.ds(8 * k, 8), :] = gated(pk(xn_rows(i, 16 * k, *ld_stats(i))), tok)

    def ay_jobs(i):
        jobs = []
        for sl in range(14):
            g = {}
            for d in range(2):
                y = dy_s[i, pl.ds(D2 * d + 16 * sl, 16), :].astype(f32)
                for t in range(2):
                    g[t, d] = y[:, 256 * t:256 * (t + 1)]
            for r, a in enumerate(spread(ALPHA, g, 2)):
                jobs.append(store_job(ay_s, (i, r, pl.ds(8 * sl, 8), slice(None)), pk(a)))
        return jobs

    def store_job(ref, idx, v):
        def run(tok):
            ref[idx] = gated(v, tok)
        return run

    def pacer(plan):
        state = {"t": 0, "done": [0] * len(plan)}

        def tick(cycles, tok, last=False):
            state["t"] += cycles
            for n, (jobs, t0, t1) in enumerate(plan):
                want = min(len(jobs), max(0, (state["t"] - t0) * len(jobs) // max(t1 - t0, 1)))
                if last:
                    want = len(jobs)
                while state["done"][n] < want:
                    jobs[state["done"][n]](tok if t1 > t0 else None)
                    state["done"][n] += 1
        return tick

    def prep_jobs(j, toks):
        jobs = []
        for w, n, ref, refT in ((wgu_s, 4, bg_s, bgT_s), (wd_s, 2, bd_s, bdT_s)):
            for r, b in enumerate(spread(BETA, grid(w[j].astype(f32), n, False), n)):
                b = b.astype(bf16)
                bT = pk(b.T)
                jobs.append(store_job(ref, r, pk(b)))
                jobs.append(store_job(refT, r, bT))
                toks.append(bT[56:64, 0:Q4])
        return jobs

    def do_units(tiles, plan, toks=(), t0=0, t1=1, extra=()):
        tick = pacer(plan)
        m = OPT_DM
        units = [(g // 4, cc, g % 4) for g in tiles for cc in range(D // m)]
        used = 0
        for n, (i, cc, t) in enumerate(units):
            lanes = pl.ds(128 * t, 128)
            w = wop_s[pl.ds(m // 2 * cc, m // 2), :]
            want = min(len(toks), max(0, (m * n - t0) * len(toks) // (t1 - t0)))
            if want > used:
                head = w[0:8]
                for tk in toks[used:want]:
                    head = jnp.concatenate([gated(head[:, 0:128], tk), head[:, 128:]], axis=1)
                w = jnp.concatenate([head, w[8:]], axis=0)
                used = want
            v = dot(up(w), dy_s[i, :, lanes])
            do_s[i, pl.ds(m * cc, m), lanes] = v
            for r in range(0, m, 56):
                tick(56, v[r:r + 8], n == len(units) - 1 and r + 56 == m)
            for at, run in extra:
                if at == n:
                    run()

    def opaque(i):
        always[0] = jax.lax.shift_right_logical(pltpu.bitcast(dy_s[i, pl.ds(0, 16), pl.ds(0, 128)], jnp.int32), 1)

    def prologue():
        first = [cp_wo(), cp_dy(0, SEM_ODD), cp_x(0, SEM_GROUP), cp_wphi(), cp_dy(1), *map(cp_wqkv, range(4)), cp_x(1)]
        for copy in first:
            copy.start()

        def clear(n, c):
            for part in range(3):
                g_acc[part, pl.ds(7 * n, 7)] = jnp.zeros((7, Q4, Q4), f32)
            return c

        jax.lax.fori_loop(0, 7, clear, 0)
        kv_acc[...] = jnp.zeros(kv_acc.shape, f32)
        dkv_acc[...] = jnp.zeros(dkv_acc.shape, f32)
        cp_wo().wait()
        wop_s[...] = pltpu.bitcast(wo_s[...], u32)
        cp_dy(0, SEM_ODD).wait()
        opaque(0)
        do_units(range(4), [(ay_jobs(0), 0, 1600)])

        bdT = []

        def phi_blocks():
            mask_cr, mask_rc, e_rf = quad_maps()
            for c in range(4):
                xq = xb_s[pl.ds(Q4 * c, Q4), :].astype(bf16)
                blk_s[c] = pk(jnp.where(mask_cr, dot(xq, e_rf, NT), 0.0))
                bdT.append(jnp.where(mask_rc, dot(e_rf, xq, NT), 0.0).astype(bf16))

        def fold_phi(d):
            wT = wqkv_s[d][...].T
            wT_s[d] = pk(wT[0:2 * D])
            for part in range(3):
                for c in range(4):
                    w = wT[D * part + Q4 * c:D * part + Q4 * (c + 1)]
                    if part < 2:
                        w = dot(bdT[c], w)
                        wf_s[c, part, d] = w
                        w = w * LOG2E
                    wpT_s[c, part, d] = pk(w)

        cp_x(0, SEM_GROUP).wait()
        cp_wphi().wait()
        cp_dy(1).wait()
        opaque(1)
        xa_s[...] = wphi_s[...].astype(f32).reshape(D, DH)
        for h in range(H):
            xb_s[pl.ds(DH * h, DH), :] = xa_s[pl.ds(h, DH, stride=H), :]
        ln = [([functools.partial(ln_stats, 0, t) for t in range(4)], OPT_P0, OPT_P1),
              ([functools.partial(ln_slab, 0, k) for k in range(D // 16)], OPT_P1, OPT_P2)]
        ay = [(ay_jobs(1), OPT_P3, OPT_P4)]
        do_units(range(4, 8), ln + ay, extra=[(OPT_PX, phi_blocks)])
        for n in range(4):
            cp_wqkv(n).wait()
        for d in range(4):
            fold_phi(d)
        cp_x(1).wait()

    prologue()

    def phase_a(i, c):
        always[0] = iota((8, 128), 0) - jnp.minimum(i, 0)
        inext = jnp.minimum(i + 1, NC - 1)

        @pl.when(i + 2 < NC)
        def _():
            cp_x(i + 2).start()
            cp_dy(i + 2).start()

        @pl.when(i < 3)
        def _():
            jw = jnp.minimum(i, 2)
            cp_wg(jw).start()
            cp_wu(jw).start()
            cp_wd(jw).start()

        seq = OPT_ASEQ
        cost = [64 if u == 4 else 112 for u in seq]
        t_xn = sum(cost[:max(n for n, u in enumerate(seq) if u < 3) + 1])
        flip = [store_job(wp_s, (i, part, d), wf_s[i, part, d].T if part < 2 else up(wpT_s[i, part, d]).T.astype(f32))
                for part in range(3) for d in range(4)]
        woT = pk(wo_s[pl.ds(pl.multiple_of(D2 * (i >> 1), D2), D2), :].T)
        flip += [store_job(woT_s, (i >> 1, pl.ds(56 * d, 56), slice(None)), woT[56 * d:56 * d + 56]) for d in range(4)]
        stats = ([functools.partial(ln_stats, inext, t) for t in range(4)], OPT_G4, OPT_G5)
        late = t_xn + OPT_G6, sum(cost) - OPT_G7
        plan = [(ax_jobs(i), OPT_G0, OPT_G1), stats,
                ([functools.partial(ln_slab, inext, k) for k in range(D // 16)], *late)]
        tick = pacer(plan + [(flip, OPT_G8, OPT_G9)])
        units = {part: [(cc, t) for cc in range(4) for t in range(4)] for part in range(3)}
        units[4] = list(range(NP))
        ph, done = {}, [None] * len(seq)
        ones = jnp.ones((8, 128), f32)
        for n, part in enumerate(seq):
            if part == 4:
                p = units[4].pop(0)
                v = dot(*[jnp.concatenate([ph[k, p, t] for t in range(4)], axis=1) for k in (2, 1)], NT)
                kv_acc[p] += v
                tick(64, v[0:8], n == len(seq) - 1)
                continue
            cc, t = units[part].pop(0)
            lanes = pl.ds(128 * t, 128)
            w = [wpT_s[cc, part, d] for d in range(4)]
            if n >= OPT_GL and done[n - OPT_GL] is not None:
                w[0] = jnp.concatenate([gated(w[0][0:8], done[n - OPT_GL]), w[0][8:]], axis=0)
            v = total([dot(up(w[d]), up(xn_s[pl.ds(Q4 // 2 * d, Q4 // 2), lanes])) for d in range(4)])
            for p in (2 * cc, 2 * cc + 1):
                z = v[PR * (p & 1):PR * (p & 1) + PR]
                z = (jnp.concatenate([z, ones], axis=0) if part == 2 else hedgehog(z)).astype(bf16)
                (phq_s, phk_s, vext_s)[part][i, p, :, lanes] = pk(z)
                ph[part, p, t] = z
            done[n] = None if part == 2 else pk(z)[24:32] | pk(ph[part, p - 1, t])[24:32]
            tick(112, v[0:8], n == len(seq) - 1)

        @pl.when(i + 2 < NC)
        def _():
            cp_x(i + 2).wait()
        return c

    jax.lax.fori_loop(0, NC, phase_a, 0)

    def bridge():
        cp_wg(0).wait()
        cp_wu(0).wait()
        cp_wd(0).wait()
        cp_dy(2).wait()
        cp_dy(3).wait()
        opaque(2)
        m_full, m_single = kv_masks()
        jobs = []
        for p in range(NP):
            kv = kv_acc[p]
            jobs.append(store_job(kvm_s, p, pk(jnp.where(m_full, kv, 0.0))))
            jobs.append(store_job(kvT_s, p, pk(jnp.where(m_single, kv, 0.0).T)))
        toks = []
        prep = prep_jobs(0, toks)
        do_units(range(8, 16), [(prep, OPT_Q0, OPT_Q1), (ay_jobs(2) + ay_jobs(3), OPT_Q2, OPT_Q3), (jobs, OPT_Q4, OPT_Q5)],
                 toks, OPT_Q6, OPT_Q7)

    bridge()

    g_order = tuple(int(t[1]) for t in OPT_FO.split() if t[0] == "g")
    d_order = tuple(int(t[1]) for t in OPT_FO.split() if t[0] == "d")

    def phase_f(j, c):
        always[0] = iota((8, 128), 0) - jnp.minimum(j, 0)
        jn = jnp.minimum(j + 1, NF - 1)

        @pl.when(j + 1 < NF)
        def _():
            cp_wg(jn).wait()
            cp_wu(jn).wait()
            cp_wd(jn).wait()

        @pl.when(j + 3 < NF)
        def _():
            jw = jnp.minimum(j + 3, NF - 1)
            cp_wg(jw).start()
            cp_wu(jw).start()
            cp_wd(jw).start()

        cg = [[[] for _ in range(49)] for _ in range(NC)]
        cd = [[[] for _ in range(7)] for _ in range(NC)]
        cs = {}

        def forward(i, m):
            rows = pl.ds(m * MS // 2, MS // 2)
            mg, md = [None] * 49, [None] * 7
            for t in OPT_FO.split():
                a = int(t[1])
                if t[0] == "g":
                    for b in OPT_FI:
                        r = 7 * a + b
                        mg[r] = dot(up(bgT_s[r, rows, :]), up(ax_s[i, r]))
                else:
                    md[a] = dot(up(bdT_s[a, rows, :]), up(ay_s[i, a]))
            gu = gather(GAMMA, mg, 4, (g_order, OPT_FI))
            dh = gather(GAMMA, md, 2, (d_order,))
            dgu, hh = {}, {}
            for t in range(4):
                for f in range(2):
                    lanes = slice(128 * (t & 1), 128 * (t & 1) + 128)
                    hh[t, f], dgu[t, f], dgu[t, f + 2] = geglu_fwd_bwd(
                        gu[t, f], gu[t, f + 2], dh[t >> 1, f][:, lanes])
            h2 = {(t, f): jnp.concatenate([hh[2 * t, f], hh[2 * t + 1, f]], axis=1)
                  for t in range(2) for f in range(2)}
            for r, a in enumerate(spread(GAMMA, dgu, 4)):
                cg[i][r].append(a.astype(bf16))
            for r, a in enumerate(spread(GAMMA, h2, 2)):
                cd[i][r].append(a.astype(bf16))
            if m == 128 // MS - 1:
                cs[i] = ([jnp.concatenate(l, axis=0).astype(bf16) for l in cg[i]],
                         [jnp.concatenate(l, axis=0).astype(bf16) for l in cd[i]])

        def prev(v):
            return jnp.where(iota(v.shape, 0) < jnp.minimum(j, 1) * 256, v, 0.0)

        def back_x(i, k):
            for n in range(XCUT[k], XCUT[k + 1]):
                if n < 7:
                    acco[i, n] = prev(acco[i, n]) + dot(up(bd_s[n]), cs[i][1][n])
                else:
                    accx[i, n - 7] = prev(accx[i, n - 7]) + dot(up(bg_s[n - 7]), cs[i][0][n - 7])

        qs = [[], []]
        toks = []
        clock = {"now": 0, "used": 0}

        def lhs(v):
            want = min(len(toks), max(0, (clock["now"] - OPT_F4) * len(toks) // (OPT_F5 - OPT_F4)))
            if want == clock["used"]:
                return up(v)
            clock["used"] = want
            return up(jnp.concatenate([gated(v[0:8], toks[want - 1]), v[8:]], axis=0))

        def back_w(h, k, tick):
            for n in range(WCUT[k], WCUT[k + 1]):
                ref, c, r = (ax_s, 0, n) if n < 49 else (ay_s, 1, n - 49)
                qs[h].append(total([dot(lhs(ref[i, r]), cs[i][c][r], NT) for i in (2 * h, 2 * h + 1)]))
                clock["now"] += 56 if n < 49 else 224
                tick(56 if n < 49 else 224, qs[h][-1][0:8], n == 55)

        def side_jobs():
            jobs = []
            r16 = pl.ds(pl.multiple_of(16 * j, 16), 16)
            r8 = pl.ds(pl.multiple_of(8 * j, 8), 8)
            for part in range(3):
                g = {(d, cc): wp_s[cc, part, d, r16, :] for d in range(4) for cc in range(4)}
                for r, b in enumerate(spread(BETA, g, 4)):
                    jobs.append(store_job(bq_s, (part, r, r8, slice(None)), pk(b)))
            g = {(d, cc): up(woT_s[cc, pl.ds(pl.multiple_of(Q4 * d + 16 * j, 16), 16), :]).astype(f32)
                 for d in range(2) for cc in range(2)}
            for r, b in enumerate(spread(BETA, g, 2)):
                jobs.append(store_job(bo_s, (r, pl.ds(pl.multiple_of(16 * j, 16), 16), slice(None)), pk(b)))
            return jobs

        ticks = [pacer([(side_jobs(), OPT_F0, OPT_F1)]), pacer([])]
        for u in OPT_FS.split():
            if u == "p":
                for job in prep_jobs(jn, toks):
                    job(None)
                clock["now"] = 0
            else:
                for k in u[2:]:
                    if u[0] == "w":
                        back_w(int(u[1]), int(k), ticks[int(u[1])])
                    else:
                        (forward if u[0] == "f" else back_x)(int(u[1]), int(k))
        q = [a + b for a, b in zip(*qs)]
        dwgu_s[j] = ungrid(gather(BETA, q[0:49], 4), 4, False).astype(bf16)
        dwd_s[j] = ungrid(gather(BETA, q[49:56], 2), 2, False).astype(bf16)
        cp_dwg(j).start()
        cp_dwu(j).start()
        cp_dwd(j).start()
        return c

    jax.lax.fori_loop(0, NF, phase_f, 0)

    def spread_slabs(pc):
        blk = {(t, cc): jnp.concatenate([pc[2 * cc, t], pc[2 * cc + 1, t]], axis=0) for t in range(4) for cc in range(4)}
        out = [[] for _ in range(49)]
        for sl in range(7):
            g = {k: v[16 * sl:16 * sl + 16] for k, v in blk.items()}
            for r, a in enumerate(spread(GAMMA, g, 4)):
                out[r].append(a.astype(bf16))
        return [jnp.concatenate(l, axis=0).astype(bf16) for l in out]

    def acc_g(i, part, cm):
        for r in range(49):
            g_acc[part, r] += dot(cm[r], up(ax_s[i, r]), NT)

    def phase_b(i, c):
        always[0] = iota((8, 128), 0) - jnp.minimum(i, 0)
        low = iota((8, 128), 0) < 4
        _, m_single = kv_masks()
        os_, dnes, dps, co, toks = {}, {}, {}, {}, []

        def num(p):
            nes = dot(up(kvm_s[p]), up(phq_s[i, p]))
            for t in range(4):
                ne = nes[:, 128 * t:128 * t + 128]
                r = 1.0 / (ne[PR:64] + 1e-6)
                rr = pltpu.roll(r, 4, 0)
                ra = jnp.where(low, r, rr)
                rb = jnp.where(low, rr, r)
                rfull = jnp.concatenate([ra, ra, ra, r, rb, rb, rb], axis=0)
                o = ne[0:PR] * rfull
                dnum = do_s[i, pl.ds(PR * p, PR), pl.ds(128 * t, 128)] * rfull
                z = dnum * o
                sa = z[0:8] + z[8:16] + z[16:24]
                sb = z[32:40] + z[40:48] + z[48:56]
                w = jnp.where(low, sa, sb) + pltpu.roll(jnp.where(low, sb, sa), 4, 0) + z[24:32]
                w = w + pltpu.roll(w, 1, 0)
                w = w + pltpu.roll(w, 2, 0)
                os_[p, t] = o
                dnes[p, t] = jnp.concatenate([dnum, -w], axis=0).astype(bf16)

        def dphi(p):
            for t in range(4):
                v = dot(up(kvT_s[p]), dnes[p, t])
                dps[p, t] = hedgehog_bwd(up(phq_s[i, p, :, pl.ds(128 * t, 128)]).astype(f32), v)

        def dkv(p):
            v = dkv_acc[p] + dot(jnp.concatenate([dnes[p, t] for t in range(4)], axis=1), up(phq_s[i, p]), NT)
            dkv_acc[p] = v
            v = jnp.where(m_single, v, 0.0)
            vT = pk(v.T)
            dkvm_s[p] = pk(v)
            dkvT_s[p] = vT
            toks.append(vT[48:56])

        def spread_o(nh):
            blk = {(t, cc): jnp.concatenate([os_[4 * cc + k, 2 * t + nh] for k in range(4)], axis=0)
                   for t in range(2) for cc in range(2)}
            parts = [[] for _ in range(7)]
            for sl in range(14):
                for r, a in enumerate(spread(GAMMA, {k: v[16 * sl:16 * sl + 16] for k, v in blk.items()}, 2)):
                    a = a.astype(bf16)
                    co_s[i, r, pl.ds(8 * sl, 8), pl.ds(128 * nh, 128)] = pk(a)
                    parts[r].append(a)
            for r in range(7):
                co[r, nh] = jnp.concatenate(parts[r], axis=0).astype(bf16)

        def out_rows(tot, r0, ms, nh):
            for (t, d), v in gather(ALPHA, tot, 2, (OPT_BO,)).items():
                rows, lanes = pl.ds(D2 * d + r0, ms), pl.ds(256 * t + 128 * nh, 128)
                out_s[i, rows, lanes] = (x_s[i, rows, lanes].astype(f32) + v).astype(bf16)

        def attn(nh, r0, ms):
            tot = [None] * 7
            if not co:
                spread_o(0)
                spread_o(1)
            for r in OPT_BO:
                rhs = co[r, nh]
                at = (i, r, pl.ds(r0, ms), pl.ds(128 * nh, 128))
                tot[r] = acco[at] + dot(up(bo_s[r, pl.ds(r0 // 2, ms // 2), :]), rhs)
            out_rows(tot, r0, ms, nh)

        units = {"n": [functools.partial(num, p) for p in OPT_BP],
                 "d": [functools.partial(dphi, p) for p in OPT_BQ],
                 "k": [functools.partial(dkv, p) for p in OPT_BP],
                 "a": [functools.partial(attn, nh, sum(OPT_BM[:n]), OPT_BM[n]) for nh in range(2) for n in range(len(OPT_BM))]}
        for u in OPT_BS:
            if units[u]:
                units[u].pop(0)()
        assert not any(units.values())
        cq = spread_slabs(dps)
        for r in range(49):
            accx[i, r] += dot(up(bq_s[0, r]), cq[r])
        for r in range(49):
            w = ax_s[i, r]
            if OPT_BR and r >= OPT_BR and (r - OPT_BR) % OPT_BT == 0 and toks:
                w = jnp.concatenate([gated(w[0:8], toks.pop(0)), w[8:]], axis=0)
            g_acc[0, r] += dot(cq[r], up(w), NT)
        cp_out(i).start()
        return c

    jax.lax.fori_loop(0, NC, phase_b, 0)

    def phase_c(i, c):
        always[0] = iota((8, 128), 0) - jnp.minimum(i, 0)
        dv, dpk = {}, {}
        for p in PAIRS:
            v = dot(up(dkvm_s[p]), up(phk_s[i, p]))
            for t in range(4):
                dv[p, t] = v[0:PR, 128 * t:128 * t + 128]
        for p in PAIRS:
            for t in range(4):
                lanes = pl.ds(128 * t, 128)
                dphi = dot(up(dkvT_s[p]), up(vext_s[i, p, :, lanes]))
                dpk[p, t] = hedgehog_bwd(up(phk_s[i, p, :, lanes]).astype(f32), dphi)

        def dwo_half(rs):
            for r in rs:
                old = dwo_acc[r]
                old = jnp.where(iota(old.shape, 0) < jnp.minimum(i, 1) * 256, old, 0.0)
                dwo_acc[r] = old + dot(up(co_s[i, r, pl.ds(0, Q4 // 2), :]), up(ay_s[i, r]), NT)

        dwo_half(range(0, OPT_C0))
        cv = spread_slabs(dv)
        acc_g(i, 2, cv)
        dwo_half(range(OPT_C0, OPT_C1))
        ck = spread_slabs(dpk)
        s1, s2 = [[] for _ in range(4)], [[] for _ in range(4)]
        r0 = 0
        for ms in OPT_CM:
            tot = [None] * 49
            half = pl.ds(r0 // 2, ms // 2)
            for a in OPT_CO:
                for b in OPT_CI:
                    r = 7 * a + b
                    tot[r] = accx[i, r, pl.ds(r0, ms), :] + (
                        dot(up(bq_s[2, r, half, :]), cv[r]) + dot(up(bq_s[1, r, half, :]), ck[r]))
            for (t, d), v in gather(ALPHA, tot, 4, (OPT_CO, OPT_CI)).items():
                rows, lanes = pl.ds(Q4 * d + r0, ms), pl.ds(128 * t, 128)
                do_s[i, rows, lanes] = v
                w = v * x_s[i, rows, lanes].astype(f32)
                s1[t].append(total([v[k:k + 8] for k in range(0, ms, 8)]))
                s2[t].append(total([w[k:k + 8] for k in range(0, ms, 8)]))
            r0 += ms
        jobs = []
        for t in range(4):
            lanes = pl.ds(128 * t, 128)
            mu, rstd = stat_s[i, 0, :, lanes], stat_s[i, 1, :, lanes]
            m1 = jnp.sum(total(s1[t]), axis=0, keepdims=True) * (1.0 / D)
            m2 = (jnp.sum(total(s2[t]), axis=0, keepdims=True) * (1.0 / D) - mu * m1) * rstd
            cb = -(rstd * rstd) * m2
            cc = -(rstd * m1) - cb * mu
            ca, cb, cc = [jnp.concatenate([z, z], axis=0) for z in (rstd, cb, cc)]

            def dx_job(rows, lanes, ca, cb, cc, tok):
                v = (dy_s[i, rows, lanes].astype(f32) + cc) + (ca * do_s[i, rows, lanes] + cb * x_s[i, rows, lanes].astype(f32))
                dx_s[i, rows, lanes] = gated(v, tok).astype(bf16)
            for k in range(D // 16):
                jobs.append(functools.partial(dx_job, pl.ds(16 * k, 16), lanes, ca, cb, cc))
        dwo_half(range(OPT_C1, 7))
        tick = pacer([(jobs, OPT_C2, OPT_C3)])
        for r in range(49):
            v = dot(ck[r], up(ax_s[i, r]), NT)
            g_acc[1, r] += v
            tick(28, v[0:8], r == 48)
        cp_dx(i).start()
        return c

    jax.lax.fori_loop(0, NC, phase_c, 0)

    def epilogue():
        def dwo_store(m, q):
            g = gather(BETA, q, 2)
            for cc in range(2):
                dwo_s[2 * cc + m][...] = jnp.concatenate([g[0, cc], g[1, cc]], axis=1).astype(bf16)
                cp_dwo(2 * cc + m).start()

        mask_cr, _, e_rf = quad_maps()
        always[0] = jax.lax.shift_right_logical(pltpu.bitcast(stat_s[0, 1, :, pl.ds(0, 128)], jnp.int32), 1)
        gT = [gather(BETA, [g_acc[part, r] for r in range(49)], 4) for part in range(3)]
        q1 = [[] for _ in range(7)]
        fill = [(r, i) for r in OPT_EO for i in range(NC)]
        blocks = [(d, part, cc) for d in range(4) for part in range(2) for cc in range(4)]
        dwT, acc = {}, [[] for _ in range(4)]
        tok = None
        for u in OPT_ES:
            if u == "f":
                r, i = fill.pop(0)
                v = dot(up(co_s[i, r, pl.ds(Q4 // 2, Q4 // 2), :]), up(ay_s[i, r]), NT)
                q1[r].append(v)
                tok = v[0:8, 0:128]
            elif u == "o":
                dwo_store(0, [gated(dwo_acc[r], tok) for r in range(7)])
            elif u == "p":
                for cc in range(4):
                    xb_s[pl.ds(Q4 * cc, Q4), :] = dot(jnp.where(mask_cr, total(acc[cc]), 0.0).astype(bf16), e_rf)
                for d in range(DH):
                    dwphi_s[d] = xb_s[pl.ds(d, H, stride=DH), :].astype(bf16)
                cp_dwphi().start()
            else:
                d, part, cc = blocks.pop(0)
                g = gT[part][d, cc].astype(bf16)
                dwT[part, cc] = dot(up(blk_s[cc]), g).astype(bf16)
                acc[cc].append(dot(up(wT_s[d, pl.ds((D * part + Q4 * cc) // 2, Q4 // 2), :]), g, NT))
                if part == 0:
                    dwT[2, cc] = gated(gT[2][d, cc], tok).astype(bf16)
                if part == 1 and cc == 3:
                    col = [dwT[k, n] for k in range(3) for n in range(4)]
                    dwq_s[d][...] = jnp.concatenate(col, axis=0).T
                    cp_dwqkv(d).start()
        assert not fill and not blocks
        dwo_store(1, [total(q) for q in q1])

    epilogue()


    for j in range(NF):
        cp_dwg(j).wait()
        cp_dwu(j).wait()
        cp_dwd(j).wait()
    for i in range(NC):
        cp_out(i).wait()
        cp_dx(i).wait()
    cp_dwphi().wait()
    for m in range(4):
        cp_dwqkv(m).wait()
        cp_dwo(m).wait()


@jax.jit
def pallas_parallel_sum__linear_kernel_hedgehog__glu_gated_geglu__prompt_kernel(
    A_x: jax.Array,
    A_wqkv: jax.Array,
    A_w_phi: jax.Array,
    A_wo: jax.Array,
    B_x: jax.Array,
    B_w_gate: jax.Array,
    B_w_up: jax.Array,
    B_w_down: jax.Array,
    grad_out: jax.Array,
):
    del B_x
    sds = jax.ShapeDtypeStruct
    vm = pltpu.VMEM
    hbm = pl.BlockSpec(memory_space=pl.ANY)
    scratch = [
        vm((NC, D, TC), bf16), vm((NC, D, TC), bf16), [vm((Q4, 3 * D), bf16)] * 4, vm((DH, H, DH), bf16),
        vm((D, D), bf16), vm((NF, D, 2 * FC), bf16), vm((NF, D, FC), bf16),
        vm((NC, D, TC), bf16), vm((NC, D, TC), bf16), [vm((Q4, 3 * D), bf16)] * 4, vm((DH, H, DH), bf16),
        [vm((Q4, D), bf16)] * 4, vm((NF, D, 2 * FC), bf16), vm((NF, D, FC), bf16),
        vm((NC, 64, 56, 128), u32), vm((NC, 8, 112, 256), u32), vm((NC, 8, 112, 256), u32),
        vm((NC, 8, 8, TC), f32), vm((NC, D, TC), f32),
        vm((NC, NP, 56, TC), u32), vm((NC, NP, 56, TC), u32), vm((NC, NP, 32, TC), u32),
        vm((NC, 64, Q4, 128), f32), vm((NC, 8, D2, 256), f32), vm((3, 49, Q4, Q4), f32),
        vm((NP, 64, 112), f32), vm((NP, 64, 112), f32),
        vm((NP, 32, 112), u32), vm((NP, 56, 64), u32), vm((NP, 32, 112), u32), vm((NP, 56, 64), u32),
        vm((49, 56, 128), u32), vm((49, 64, Q4), u32), vm((7, 112, 128), u32), vm((7, 64, D2), u32),
        vm((3, 49, 56, Q4), u32), vm((7, 112, D2), u32),
        vm((4, D, Q4), u32), vm((4, 56, Q4), u32), vm((D, DH), f32), vm((D, DH), f32),
        vm((D2, TC), u32), vm((D2, D), u32), vm((4, 4, 4, 56, Q4), u32), vm((4, 4, 4, Q4, Q4), f32), vm((2, D2, D2), u32),
        vm((4, 2, 4, Q4, Q4), f32),
        vm((7, Q4, D2), f32),
        pltpu.SemaphoreType.DMA((NSEM,)),
    ]
    outs = pl.pallas_call(
        kernel,
        in_specs=[hbm] * 8,
        out_specs=[hbm] * 8,
        out_shape=[sds((D, S), bf16), sds((D, S), bf16), sds((D, 3 * D), bf16), sds((DH, H, DH), bf16),
                   sds((D, D), bf16), sds((D, F), bf16), sds((D, F), bf16), sds((D, F), bf16)],
        scratch_shapes=scratch,
        compiler_params=pltpu.CompilerParams(vmem_limit_bytes=110 * 1024 * 1024),
        name="hedgehog_geglu_fwd_bwd",
    )(A_x[0].T, grad_out[0].T, A_wqkv, A_w_phi.transpose(1, 0, 2), A_wo, B_w_gate, B_w_up, B_w_down.T)
    outT, dxT, dwqkv, dwphi, dwo, dwg, dwu, dwdT = outs
    return (outT.T[None], dxT.T[None], dwqkv, dwphi.transpose(1, 0, 2), dwo, dwg, dwu, dwdT.T)
```
